```python
import jax
import jax.numpy as jnp

def _softmax(x, axis=-1):
    return jax.nn.softmax(x, axis=axis)
def _gelu(x):
    return jax.nn.gelu(x, approximate=True)
def _silu(x):
    return jax.nn.silu(x)
def _sigmoid(x):
    return jax.nn.sigmoid(x)
def _layernorm(x, axis=-1, eps=1e-5):
    m = jnp.mean(x, axis=axis, keepdims=True)
    v = jnp.var(x, axis=axis, keepdims=True)
    return (x - m) / jnp.sqrt(v + eps)
def _scatter_add(tgt, idx, src, axis=0):
    return tgt.at[idx].add(src)
def _segment_sum(src, seg, n):
    return jax.ops.segment_sum(src, seg, n)
class _Rng:
    def __init__(self, key):
        self._k = key
    def _next(self):
        self._k, sub = jax.random.split(self._k)
        return sub
    def normal(self, shape):
        return jax.random.normal(self._next(), shape, dtype=jnp.bfloat16)
    def randint(self, lo, hi, shape):
        return jax.random.randint(self._next(), shape, lo, hi, dtype=jnp.int32)
    def uniform(self, shape, lo=0.0, hi=1.0):
        return jax.random.uniform(self._next(), shape, jnp.bfloat16, lo, hi)
    def permutation(self, n):
        return jax.random.permutation(self._next(), n)


kernel_name = 'standalone__modern_conv_block_convnext_v2__vision'

def setup_inputs():
    _rng = _Rng(jax.random.key(int.from_bytes(__import__("os").urandom(4), "little")))
    _w = (lambda a: (lambda t: t.astype(jnp.bfloat16) if jnp.issubdtype(t.dtype, jnp.floating) else t)(jnp.asarray(a)))
    H = W = 512
    C = 96
    K = 3
    return {
        "x": _w((lambda *s: _rng.normal(s) * 0.05)(1, H, W, C)),
        "dw": _w((lambda *s: _rng.normal(s) * 0.05)(K, K, C)),
        "w1": _w((lambda *s: _rng.normal(s) * 0.05)(C, 4 * C)),
        "w2": _w((lambda *s: _rng.normal(s) * 0.05)(4 * C, C)),
        "grn_gamma": _w((lambda *s: _rng.normal(s) * 0.05)(4 * C)),
        "grn_beta": _w((lambda *s: _rng.normal(s) * 0.05)(4 * C)),
    }

def reference(x, dw, w1, w2, grn_gamma, grn_beta):
    B, H, W, C = x.shape
    K = dw.shape[0]
    pad = K // 2
    xp = jnp.pad(x, ((0,0),(pad,pad),(pad,pad),(0,0)))
    out = jnp.zeros_like(x)
    for i in range(K):
        for j in range(K):
            out = out + xp[:, i:i+H, j:j+W, :] * dw[i, j][None, None, None, :]
    h = _layernorm(out, axis=-1)
    h = jnp.einsum('bhwc,ce->bhwe', h, w1)
    h = _gelu(h)
    gx = jnp.sqrt((h * h).sum(axis=(1, 2), keepdims=True) + 1e-6)
    nx = gx / (gx.mean(axis=-1, keepdims=True) + 1e-6)
    h = grn_gamma * (h * nx) + grn_beta + h
    h = jnp.einsum('bhwe,ec->bhwc', h, w2)
    return x + h
```

```python
import jax
import jax.numpy as jnp
import numpy as np
import jax.experimental.pallas as pl
import jax.experimental.pallas.tpu as pltpu

_C0 = float(np.sqrt(2.0 / np.pi))
_ALPHA = float((_C0 * 0.044715) ** (1.0 / 3.0))
_A = _C0 / _ALPHA
U1 = 2
U2 = 2
TH = 8
NS = 4

def make(H, W, C, E):
    NB = H // TH
    G = C // 8
    NP = H // 2
    f32, bf16, u32 = jnp.float32, jnp.bfloat16, jnp.uint32

    def kern(x_hbm, dw_ref, w1_ref, w2t_ref, g_ref, b_ref, o_hbm,
             xb, hs, ls, lt, S, w1t, w2s, L, acc, bias, isem, osem, psem):
        def in1(b):
            slot = b % NS
            return pltpu.make_async_copy(x_hbm.at[pl.ds(b * TH + 3, TH)], xb.at[slot], isem.at[slot])
        def in1_last():
            slot = (NB - 1) % NS
            return pltpu.make_async_copy(x_hbm.at[pl.ds((NB - 1) * TH + 3, TH - 3)], xb.at[slot, pl.ds(0, TH - 3)], isem.at[slot])
        def in0():
            return pltpu.make_async_copy(x_hbm.at[pl.ds(0, 3)], xb.at[NS - 1, pl.ds(0, 3)], psem.at[0])
        def in2(b):
            slot = b % NS
            return pltpu.make_async_copy(x_hbm.at[pl.ds(b * TH, TH)], xb.at[slot], isem.at[slot])
        def out2(b):
            slot = b % NS
            return pltpu.make_async_copy(xb.at[slot], o_hbm.at[pl.ds(b * TH, TH)], osem.at[slot])

        in0().start()
        in1(0).start()
        in1(1).start()

        w1t[0] = w1_ref[...].astype(f32).T.astype(bf16)
        dwt = dw_ref[...].astype(f32).T
        ri = jax.lax.broadcasted_iota(jnp.int32, (8, 96), 0)
        ci = jax.lax.broadcasted_iota(jnp.int32, (8, 96), 1)
        for g in range(G):
            rows = []
            for o in range(2):
                m = jnp.zeros((8, 96), f32)
                for j in range(3):
                    for i in range(o, o + 3):
                        p, hf = i // 2, i % 2
                        if g % 2 == 1:
                            hf = 1 - hf
                        col0 = j * 32 + p * 16 + hf * 8
                        k = (i - o) * 3 + j
                        m = jnp.where(ci - col0 == ri, dwt[8 * g:8 * g + 8, k:k + 1], m)
                rows.append(m)
            L[g] = jnp.concatenate(rows, axis=0).astype(bf16)
        acc[...] = jnp.zeros_like(acc)

        sub = jax.lax.broadcasted_iota(jnp.int32, (8, W), 0)
        lane = jax.lax.broadcasted_iota(jnp.int32, (8, W), 1)
        lo = sub < 4
        first = lane == 0
        last = lane == W - 1

        def prep(a, b):
            a = pltpu.bitcast(a, u32)
            b = pltpu.roll(pltpu.bitcast(b, u32), 4, 0)
            res = []
            for p in (jnp.where(lo, a, b), jnp.where(lo, b, a)):
                l = jnp.where(first, jnp.uint32(0), pltpu.roll(p, 1, 1))
                r = jnp.where(last, jnp.uint32(0), pltpu.roll(p, W - 1, 1))
                res.append([pltpu.bitcast(t, bf16) for t in (l, p, r)])
            return res

        def conv_ln(ra, rb):
            ys = [[], []]
            for q in range(G // 2):
                new2 = prep(ra[pl.ds(16 * q, 16), :], rb[pl.ds(16 * q, 16), :])
                for e in range(2):
                    g = 2 * q + e
                    new = new2[e]
                    parts = []
                    for j in range(3):
                        parts += [S[g, j], new[j]]
                    for j in range(3):
                        S[g, j] = new[j]
                    y = jnp.dot(L[g], jnp.concatenate(parts, axis=0), preferred_element_type=f32)
                    ys[0].append(y[0:8]); ys[1].append(y[8:16])
            outs = []
            for y in ys:
                s1 = y[0]; s2 = y[0] * y[0]
                for t in y[1:]:
                    s1 = s1 + t; s2 = s2 + t * t
                m = jnp.sum(s1, axis=0, keepdims=True) * (1.0 / C)
                v = jnp.maximum(jnp.sum(s2, axis=0, keepdims=True) * (1.0 / C) - m * m, 0.0)
                r = jax.lax.rsqrt(v + 1e-5) * _ALPHA
                outs.append(((jnp.concatenate(y, axis=0) - m) * r).astype(bf16))
            return outs

        def gelu(z):
            t = jnp.tanh(z * (z * z + _A))
            return z * t + z

        def mlp1(l, store):
            g = gelu(jnp.dot(w1t[0], l, preferred_element_type=f32))
            if store is not None:
                hs[store] = g.astype(bf16)
            g2 = g * g
            s = g2[:, 0:128]
            for t in range(1, W // 128):
                s = s + g2[:, t * 128:(t + 1) * 128]
            acc[...] += s

        in0().wait()
        for q in range(G // 2):
            new2 = prep(jnp.zeros((16, W), bf16), xb[NS - 1, 0, pl.ds(16 * q, 16), :])
            for e in range(2):
                for j in range(3):
                    S[2 * q + e, j] = new2[e][j]
        la, lb = conv_ln(xb.at[NS - 1, 1], xb.at[NS - 1, 2])
        lt[0] = la; lt[1] = lb; ls[0] = lb

        def p1_block(b, _):
            slot = b % NS
            @pl.when(b + 2 < NB - 1)
            def _():
                in1(b + 2).start()
            @pl.when(b + 2 == NB - 1)
            def _():
                in1_last().start()
                xb[(NB - 1) % NS, pl.ds(TH - 3, 3)] = jnp.zeros((3, C, W), bf16)
            @pl.when(b < NB - 1)
            def _():
                in1(b).wait()
            @pl.when(b == NB - 1)
            def _():
                in1_last().wait()
            def body(it, _):
                la, lb = lt[0], lt[1]
                for u in range(U1):
                    kk = it * U1 + u
                    k = b * (TH // 2) + kk
                    mlp1(la, k)
                    na, nb = conv_ln(xb.at[slot, 2 * kk], xb.at[slot, 2 * kk + 1])
                    mlp1(lb, None)
                    ls[k + 1] = nb
                    la, lb = na, nb
                lt[0] = la; lt[1] = lb
                return 0
            n_it = TH // 2 // U1
            if n_it == 1:
                body(0, 0)
            else:
                jax.lax.fori_loop(0, n_it, body, 0)
            return 0
        jax.lax.fori_loop(0, NB, p1_block, 0)

        in2(0).start()
        in2(1).start()
        sc = 1.0 / (2.0 * _ALPHA)
        ss = jnp.sum(acc[...].T, axis=0, keepdims=True) * (sc * sc)
        gx = jnp.sqrt(ss + 1e-6)
        nx = gx / (jnp.mean(gx, axis=-1, keepdims=True) + 1e-6)
        s = (g_ref[...].astype(f32) * nx + 1.0) * sc
        w2f = w2t_ref[...].astype(f32)
        w2s[0] = (w2f * s).astype(bf16)
        bias[...] = jnp.broadcast_to(jnp.sum(w2f * b_ref[...].astype(f32), axis=1, keepdims=True), (C, 128))

        def p2_block(b, _):
            slot = b % NS
            @pl.when(b + 2 < NB)
            def _():
                @pl.when(b + 2 >= NS)
                def _():
                    out2(b + 2 - NS).wait()
                in2(b + 2).start()
            in2(b).wait()
            def fin(h, r):
                o = jnp.dot(w2s[0], h, preferred_element_type=f32)
                o = o + jnp.tile(bias[...], (1, W // 128)) + xb[slot, r].astype(f32)
                xb[slot, r] = o.astype(bf16)
            def body(it, _):
                for u in range(U2):
                    kk = it * U2 + u
                    k = b * (TH // 2) + kk
                    g = gelu(jnp.dot(w1t[0], ls[k], preferred_element_type=f32)).astype(bf16)
                    fin(hs[k], 2 * kk)
                    fin(g, 2 * kk + 1)
                return 0
            n_it = TH // 2 // U2
            if n_it == 1:
                body(0, 0)
            else:
                jax.lax.fori_loop(0, n_it, body, 0)
            out2(b).start()
            return 0
        jax.lax.fori_loop(0, NB, p2_block, 0)
        for b in range(NB - NS, NB):
            out2(b).wait()
    return kern

@jax.jit
def pallas_standalone__modern_conv_block_convnext_v2__vision_kernel(x, dw, w1, w2, grn_gamma, grn_beta):
    B, H, W, C = x.shape
    E = w1.shape[1]
    xt = jnp.transpose(x[0], (0, 2, 1))
    vm = pl.BlockSpec(memory_space=pltpu.VMEM)
    bf16 = jnp.bfloat16
    out = pl.pallas_call(
        make(H, W, C, E),
        in_specs=[pl.BlockSpec(memory_space=pl.ANY), vm, vm, vm, vm, vm],
        out_specs=pl.BlockSpec(memory_space=pl.ANY),
        out_shape=jax.ShapeDtypeStruct((H, C, W), x.dtype),
        scratch_shapes=[
            pltpu.VMEM((NS, TH, C, W), bf16),
            pltpu.VMEM((H // 2, E, W), bf16),
            pltpu.VMEM((H // 2 + 1, C, W), bf16),
            pltpu.VMEM((2, C, W), bf16),
            pltpu.VMEM((C // 8, 3, 16, W), bf16),
            pltpu.VMEM((1, E, C), bf16),
            pltpu.VMEM((1, C, E), bf16),
            pltpu.VMEM((C // 8, 16, 96), bf16),
            pltpu.VMEM((E, 128), jnp.float32),
            pltpu.VMEM((C, 128), jnp.float32),
            pltpu.SemaphoreType.DMA((NS,)),
            pltpu.SemaphoreType.DMA((NS,)),
            pltpu.SemaphoreType.DMA((1,)),
        ],
        compiler_params=pltpu.CompilerParams(vmem_limit_bytes=127 * 1024 * 1024),
    )(xt, dw.reshape(9, C), w1, w2.T, grn_gamma.reshape(1, E), grn_beta.reshape(1, E))
    return jnp.transpose(out, (0, 2, 1))[None]
```

```python
import jax
import jax.numpy as jnp
import numpy as np
import jax.experimental.pallas as pl
import jax.experimental.pallas.tpu as pltpu

_C0 = float(np.sqrt(2.0 / np.pi))
_ALPHA = float((_C0 * 0.044715) ** (1.0 / 3.0))
_A = _C0 / _ALPHA
U1 = 8
U2 = 8
NS1 = 2
NS2 = 3
ORD = 'accbcc'
GS = 2
AR = 0
LR = 12
LS = 1
CP = 0
GV = 1
SV = 0
FC = 1

def make(H, W, C, E):
    G = C // 8
    NT = W // 128
    T1, T2 = 2 * U1, 2 * U2
    NB1, NB2 = H // T1, H // T2
    f32, bf16, u32 = jnp.float32, jnp.bfloat16, jnp.uint32
    OFF = 5
    pk = lambda v: pltpu.bitcast(v.astype(bf16), u32)
    up = lambda v: pltpu.bitcast(v, bf16)

    def gelu(z):
        t = jnp.tanh(z * (z * z + _A))
        return z * t + z if GV == 0 else (t + 1.0) * z

    def kern(x_hbm, dw_ref, w1_ref, w2t_ref, g_ref, b_ref, o_hbm, hs, ls, w1t, acc):
        def phase1(xb, lt, lu, sa, mr, S, Y, L, isem, psem):
            def in1(b):
                slot = b % NS1
                return pltpu.make_async_copy(x_hbm.at[pl.ds(b * T1 + OFF, T1)], xb.at[slot], isem.at[slot])
            def in1_last():
                slot = (NB1 - 1) % NS1
                return pltpu.make_async_copy(x_hbm.at[pl.ds((NB1 - 1) * T1 + OFF, T1 - OFF)], xb.at[slot, pl.ds(0, T1 - OFF)], isem.at[slot])
            in0 = pltpu.make_async_copy(x_hbm.at[pl.ds(0, OFF)], xb.at[NS1 - 1, pl.ds(T1 - OFF, OFF)], psem.at[0])
            in0.start()
            xb[NS1 - 1, T1 - 6] = jnp.zeros((C, W), bf16)
            for b in range(NS1 - 1 - CP):
                in1(b).start()

            w1f = w1_ref[...].astype(f32)
            if FC:
                w1f = w1f - jnp.mean(w1f, axis=0, keepdims=True)
            w1t[...] = pk(w1f.T)
            dwt = dw_ref[...].astype(f32).T
            ri = jax.lax.broadcasted_iota(jnp.int32, (8, 96), 0)
            ci = jax.lax.broadcasted_iota(jnp.int32, (8, 96), 1)
            for g in range(G):
                rows = []
                for o in range(2):
                    m = jnp.zeros((8, 96), f32)
                    for j in range(3):
                        for i in range(o, o + 3):
                            col0 = (i // 2) * 48 + j * 16 + (i % 2) * 8
                            k = (i - o) * 3 + j
                            m = jnp.where(ci - col0 == ri, dwt[8 * g:8 * g + 8, k:k + 1], m)
                    rows.append(m)
                L[g] = pk(jnp.concatenate(rows, axis=0))
            acc[...] = jnp.zeros_like(acc)

            lane = jax.lax.broadcasted_iota(jnp.int32, (8, 128), 1)
            first = lane == 0
            last = lane == 127

            def prep(rows2, g):
                p = pltpu.bitcast(rows2[:, pl.ds(8 * g, 8), :].reshape(16, W), u32)
                pt = [p[:, 128 * t:128 * (t + 1)] for t in range(NT)]
                zero = jnp.zeros((8, 128), u32)
                rl = [zero] + [pltpu.roll(v, 1, 1) for v in pt]
                rr = [pltpu.roll(v, 127, 1) for v in pt] + [zero]
                l = jnp.concatenate([jnp.where(first, rl[t], rl[t + 1]) for t in range(NT)], axis=1)
                r = jnp.concatenate([jnp.where(last, rr[t + 1], rr[t]) for t in range(NT)], axis=1)
                return [l, p, r]

            def tiles(v):
                return jnp.concatenate([v[8 * r:8 * r + 8, 128 * t:128 * (t + 1)] for r in range(2) for t in range(NT)], axis=0)

            def norm(par, g, kn):
                for r in range(2):
                    y = Y[r, pl.ds(8 * g, 8), :]
                    if not FC:
                        y = y - mr[par, 0, r]
                    v = (y * mr[par, 1, r]).astype(bf16)
                    if r == 1:
                        ls[kn, pl.ds(8 * g, 8), :] = v
                    if r == 0 or not LS:
                        lt[r, pl.ds(8 * g, 8), :] = v
                    if g % 2 == 1:
                        q = g // 2
                        src = ls.at[kn] if (r == 1 and LS) else lt.at[r]
                        lu[par, r, pl.ds(8 * q, 8), :] = pltpu.bitcast(src[pl.ds(16 * q, 16), :].reshape(2, 8, W).reshape(16, W), u32)

            def conv(prev2, rows2, g, par, kn, st):
                new = prep(rows2, g)
                if CP:
                    parts = [S[g, 0], pltpu.bitcast(prev2[:, pl.ds(8 * g, 8), :].reshape(16, W), u32), S[g, 2]] + new
                else:
                    parts = [S[g, j] for j in range(3)] + new
                for j in range(3):
                    if j != 1 or not CP:
                        S[g, j] = new[j]
                y = jnp.dot(up(L[g]), up(jnp.concatenate(parts, axis=0)), preferred_element_type=f32)
                if kn is not None:
                    norm(1 - par, g, kn)
                Y[0, pl.ds(8 * g, 8), :] = y[0:8]
                Y[1, pl.ds(8 * g, 8), :] = y[8:16]
                y = tiles(y)
                s1, s2 = (y, y * y) if g % GS == 0 else (st[0] + y, st[1] + y * y)
                if g == GS - 1:
                    sa[0] = s1; sa[1] = s2
                elif g % GS == GS - 1:
                    sa[0] += s1; sa[1] += s2
                if g == G - 1:
                    red = []
                    for i in range(2):
                        p = [sa[i, pl.ds(j, 2 * NT, stride=8), :] for j in range(8)]
                        red.append((((p[0] + p[1]) + (p[2] + p[3])) + ((p[4] + p[5]) + (p[6] + p[7]))) * (1.0 / C))
                    v = jnp.maximum(red[1] - red[0] * red[0], 0.0)
                    res = [red[0], jax.lax.rsqrt(v * (1.0 / _ALPHA ** 2) + 1e-5 / _ALPHA ** 2)]
                    for i in range(1 if FC else 0, 2):
                        for r in range(2):
                            mr[par, i, r] = jnp.concatenate([jnp.broadcast_to(res[i][r * NT + t:r * NT + t + 1], (8, 128)) for t in range(NT)], axis=1)
                return s1, s2

            def mlp1(l, m0, M, store, s):
                g = gelu(jnp.dot(up(w1t[pl.ds(m0 // 2, M // 2), :]), l, preferred_element_type=f32))
                if store is not None:
                    hs[store, pl.ds(m0, M), :] = g.astype(bf16)
                g2 = g * g
                p = [g2[:, t * 128:(t + 1) * 128] for t in range(NT)]
                if SV == 0:
                    s = p[0] if s is None else s + p[0]
                    return ((s + p[1]) + p[2]) + p[3]
                if SV == 1:
                    p = (p[0] + p[1]) + (p[2] + p[3])
                    return p if s is None else s + p
                if SV == 2:
                    acc[pl.ds(m0, M), :] += (p[0] + p[1]) + (p[2] + p[3])
                if SV == 3:
                    acc[pl.ds(m0, M), :] = (((acc[pl.ds(m0, M), :] + p[0]) + p[1]) + p[2]) + p[3]
                return None

            in0.wait()
            for g in range(G):
                new = prep(xb.at[NS1 - 1, pl.ds(T1 - 6, 2)], g)
                for j in range(3):
                    S[g, j] = new[j]
            for k in range(2):
                sts = None
                for g in range(G):
                    sts = conv(xb.at[NS1 - 1, pl.ds(T1 - 6 + 2 * k, 2)], xb.at[NS1 - 1, pl.ds(T1 - 4 + 2 * k, 2)], g, k, 0 if k == 1 else None, sts)

            def block(b, _):
                slot = b % NS1
                nb = b + NS1 - 1 - CP
                @pl.when(nb < NB1 - 1)
                def _():
                    in1(nb).start()
                @pl.when(nb == NB1 - 1)
                def _():
                    in1_last().start()
                    xb[(NB1 - 1) % NS1, pl.ds(T1 - OFF, OFF)] = jnp.zeros((OFF, C, W), bf16)
                @pl.when(b < NB1 - 1)
                def _():
                    in1(b).wait()
                @pl.when(b == NB1 - 1)
                def _():
                    in1_last().wait()
                nst = G // ORD.count('c')
                M = E // nst
                for u in range(U1):
                    k = b * U1 + u
                    prev2 = xb.at[slot, pl.ds(2 * u - 2, 2)] if u else xb.at[(b + NS1 - 1) % NS1, pl.ds(T1 - 2, 2)]
                    g = 0
                    sts = None
                    for st in range(nst):
                        ss = None
                        for what in ORD:
                            if what == 'c':
                                sts = conv(prev2, xb.at[slot, pl.ds(2 * u, 2)], g, u % 2, k + 1, sts)
                                g += 1
                            else:
                                r = 'ab'.index(what)
                                fst = ss is None
                                ss = mlp1(up(lu[u % 2, r]), st * M, M, k if r == 0 else None, ss)
                                if not fst:
                                    acc[pl.ds(st * M, M), :] += ss
                return 0
            jax.lax.fori_loop(0, NB1, block, 0)

        pl.run_scoped(
            phase1,
            pltpu.VMEM((NS1, T1, C, W), bf16),
            pltpu.VMEM((2, C, W), bf16),
            pltpu.VMEM((2, 2, C // 2, W), u32),
            pltpu.VMEM((2, 16 * NT, 128), f32),
            pltpu.VMEM((2, 2, 2, 8, W), f32),
            pltpu.VMEM((G, 3, 8, W), u32),
            pltpu.VMEM((2, C, W), f32),
            pltpu.VMEM((G, 8, 96), u32),
            pltpu.SemaphoreType.DMA((NS1,)),
            pltpu.SemaphoreType.DMA((1,)),
        )

        def phase2(xb, w2s, bias, isem, osem):
            AH = min(2, NS2 - 2)
            def in2(b):
                slot = b % NS2
                return pltpu.make_async_copy(x_hbm.at[pl.ds(b * T2, T2)], xb.at[slot], isem.at[slot])
            def out2(b):
                slot = b % NS2
                return pltpu.make_async_copy(xb.at[slot], o_hbm.at[pl.ds(b * T2, T2)], osem.at[slot])
            for b in range(AH):
                in2(b).start()
            sc = 1.0 / (2.0 * _ALPHA)
            ss = jnp.sum(acc[...].T, axis=0, keepdims=True) * (sc * sc)
            gx = jnp.sqrt(ss + 1e-6)
            nx = gx / (jnp.mean(gx, axis=-1, keepdims=True) + 1e-6)
            s = (g_ref[...].astype(f32) * nx + 1.0) * sc
            w2f = w2t_ref[...].astype(f32)
            w2s[...] = pk(w2f * s)
            bias[...] = jnp.broadcast_to(jnp.sum(w2f * b_ref[...].astype(f32), axis=1, keepdims=True), (C, 128))

            def block(b, _):
                slot = b % NS2
                @pl.when(b + AH < NB2)
                def _():
                    @pl.when(b + AH >= NS2)
                    def _():
                        out2(b + AH - NS2).wait()
                    in2(b + AH).start()
                in2(b).wait()
                def fin(h, r):
                    o = jnp.dot(up(w2s[...]), h, preferred_element_type=f32)
                    o = o + jnp.tile(bias[...], (1, NT)) + xb[slot, r].astype(f32)
                    xb[slot, r] = o.astype(bf16)
                for u in range(U2):
                    k = b * U2 + u
                    g = gelu(jnp.dot(up(w1t[...]), ls[k], preferred_element_type=f32)).astype(bf16)
                    fin(hs[k], 2 * u)
                    fin(g, 2 * u + 1)
                out2(b).start()
                return 0
            jax.lax.fori_loop(0, NB2, block, 0)
            for b in range(NB2 - NS2, NB2):
                out2(b).wait()

        pl.run_scoped(
            phase2,
            pltpu.VMEM((NS2, T2, C, W), bf16),
            pltpu.VMEM((C // 2, E), u32),
            pltpu.VMEM((C, 128), f32),
            pltpu.SemaphoreType.DMA((NS2,)),
            pltpu.SemaphoreType.DMA((NS2,)),
        )
    return kern

@jax.jit
def pallas_standalone__modern_conv_block_convnext_v2__vision_kernel(x, dw, w1, w2, grn_gamma, grn_beta):
    B, H, W, C = x.shape
    E = w1.shape[1]
    xt = jnp.transpose(x[0], (0, 2, 1))
    vm = pl.BlockSpec(memory_space=pltpu.VMEM)
    bf16, u32 = jnp.bfloat16, jnp.uint32
    out = pl.pallas_call(
        make(H, W, C, E),
        in_specs=[pl.BlockSpec(memory_space=pl.ANY), vm, vm, vm, vm, vm],
        out_specs=pl.BlockSpec(memory_space=pl.ANY),
        out_shape=jax.ShapeDtypeStruct((H, C, W), x.dtype),
        scratch_shapes=[
            pltpu.VMEM((H // 2, E, W), bf16),
            pltpu.VMEM((H // 2 + 1, C, W), bf16),
            pltpu.VMEM((E // 2, C), u32),
            pltpu.VMEM((E, 128), jnp.float32),
        ],
        compiler_params=pltpu.CompilerParams(vmem_limit_bytes=127 * 1024 * 1024),
    )(xt, dw.reshape(9, C), w1, w2.T, grn_gamma.reshape(1, E), grn_beta.reshape(1, E))
    return jnp.transpose(out, (0, 2, 1))[None]
```

```python
import functools
import jax
import jax.numpy as jnp
import numpy as np
import jax.experimental.pallas as pl
import jax.experimental.pallas.tpu as pltpu

_C0 = float(np.sqrt(2.0 / np.pi))
_ALPHA = float((_C0 * 0.044715) ** (1.0 / 3.0))
_A = _C0 / _ALPHA
U = 8
NA = 1
RF = 3
NRF = 26
NO = 4
PO = 0
PI = 0
PB = 0
K = 15
N0 = 16
NM = 0
GS = 2
PAD = 0
ISB = 0
VL = 128

def make(H, W, C, E):
    G = C // 8
    NT = W // 128
    T = 2 * U
    NB = H // T
    NL = U - NA
    NSP = RF * NRF
    QR = NB * NL - NSP
    f32, bf16, u32 = jnp.float32, jnp.bfloat16, jnp.uint32
    OFF = 5
    pk = lambda v: pltpu.bitcast(v.astype(bf16), u32)
    up = lambda v: pltpu.bitcast(v, bf16)

    def gelu(z):
        return (jnp.tanh(z * (z * z + _A)) + 1.0) * z

    def hpos(u, r):
        if u < NA:
            return 2 * u + r
        return NA + u if r == 0 else None

    def lslot(b, u):
        i = b * NL + (u - NA)
        return jnp.where(i >= QR, i - QR, i)

    def kern(x_hbm, dw_hbm, w1_hbm, w2t_hbm, g_hbm, b_hbm, o_hbm, hs, ls, xb, w1t, acc, isem, lsem, osem,
             w1_ref, w2t_ref, dw_ref, g_ref, b_ref, wsem):
        small = [pltpu.make_async_copy(s, d, wsem.at[i]) for i, (s, d) in enumerate(
            [(dw_hbm, dw_ref.at[pl.ds(0, 3)]), (w1_hbm, w1_ref), (w2t_hbm, w2t_ref), (g_hbm, g_ref), (b_hbm, b_ref)])]
        def in1(b):
            return pltpu.make_async_copy(x_hbm.at[pl.ds(b * T + OFF, T)], xb.at[b % 2], isem.at[b % 2])
        ls_ = (NB - 1) % 2
        in1_last = pltpu.make_async_copy(x_hbm.at[pl.ds((NB - 1) * T + OFF, T - OFF)], xb.at[ls_, pl.ds(0, T - OFF)], isem.at[ls_])
        in0 = pltpu.make_async_copy(x_hbm.at[pl.ds(0, OFF)], xb.at[1, pl.ds(T - OFF, OFF)], isem.at[1])
        def in2(n):
            s = (NB + n) % 2
            return pltpu.make_async_copy(x_hbm.at[pl.ds((NB - 1 - n) * T, T)], xb.at[s], isem.at[s])
        def out2(n):
            b = NB - 1 - n
            return pltpu.make_async_copy(hs.at[b, pl.ds(0, T)], o_hbm.at[pl.ds(b * T, T)], osem.at[n])
        def far(n):
            return pltpu.make_async_copy(x_hbm.at[pl.ds((NB - 1 - n) * T, T)], hs.at[NB + K + 1 - n, pl.ds(T, T)], osem.at[n])
        def near(n):
            s = (NB + n) % 2
            return pltpu.make_async_copy(hs.at[NB + K + 1 - n, pl.ds(T, T)], xb.at[s], isem.at[s])
        spill = pltpu.make_async_copy(ls.at[pl.ds(0, NSP)], o_hbm.at[pl.ds(0, NSP)], lsem.at[0])
        def back(n):
            sl = pl.ds(NSP - RF * (n + 1), RF)
            return pltpu.make_async_copy(o_hbm.at[sl], ls.at[sl], lsem.at[n % 2])

        def phase1(lu, sa, mr, S, Y, L):
            small[0].start()
            in0.start()
            for cp in small[1:]:
                cp.start()
            in1(0).start()
            xb[1, T - OFF - 1] = jnp.zeros((C, W), bf16)
            acc[...] = jnp.zeros_like(acc)
            small[0].wait()

            kr = jax.lax.broadcasted_iota(jnp.int32, (16, C), 0)
            taps = jnp.zeros((16, C), f32)
            for i in range(3):
                di = dw_ref[i].astype(f32)
                for j in range(3):
                    taps = jnp.where(kr == 3 * i + j, di[j:j + 1], taps)
            taps = taps.T.astype(bf16)
            ki = jax.lax.broadcasted_iota(jnp.int32, (16, 96), 0)
            col = jax.lax.broadcasted_iota(jnp.int32, (16, 96), 1)
            new_pair = (col >= 48).astype(jnp.int32)
            row_in = 2 * new_pair + ((col >> 3) & 1)
            shift = (col - 48 * new_pair) >> 4
            diag = (jax.lax.broadcasted_iota(jnp.int32, (C, 96), 0) & 7) == (jax.lax.broadcasted_iota(jnp.int32, (C, 96), 1) & 7)
            m = []
            for o in range(2):
                sel = jnp.logical_and(ki == (row_in - o) * 3 + shift, ki < 9).astype(f32).astype(bf16)
                m.append(jnp.where(diag, jnp.dot(taps, sel, preferred_element_type=f32), 0.0))
            for g in range(G):
                L[g] = pk(jnp.concatenate([m[0][8 * g:8 * g + 8], m[1][8 * g:8 * g + 8]], axis=0))

            lane = jax.lax.broadcasted_iota(jnp.int32, (8, 128), 1)
            first = lane == 0
            last = lane == 127

            def prep(rows2, g):
                p = pltpu.bitcast(rows2[:, pl.ds(8 * g, 8), :].reshape(16, W), u32)
                pt = [p[:, 128 * t:128 * (t + 1)] for t in range(NT)]
                zero = jnp.zeros((8, 128), u32)
                rl = [zero] + [pltpu.roll(v, 1, 1) for v in pt]
                rr = [pltpu.roll(v, 127, 1) for v in pt] + [zero]
                l = jnp.concatenate([jnp.where(first, rl[t], rl[t + 1]) for t in range(NT)], axis=1)
                r = jnp.concatenate([jnp.where(last, rr[t + 1], rr[t]) for t in range(NT)], axis=1)
                return [l, p, r]

            def tiles(v):
                return jnp.concatenate([v[8 * r:8 * r + 8, 128 * t:128 * (t + 1)] for r in range(2) for t in range(NT)], axis=0)

            held = [None, None]
            def norm(par, g, keep):
                for r in range(2):
                    if NM == 0:
                        if g % 2:
                            continue
                        y = Y[r, pl.ds(8 * g, 16), :]
                        rs = mr[par, r]
                        v = jnp.concatenate([y[0:8] * rs, y[8:16] * rs], axis=0).astype(bf16)
                    else:
                        v = Y[r, pl.ds(8 * g, 8), :] * mr[par, r]
                        if g % 2 == 0:
                            held[r] = v
                            continue
                        v = jnp.concatenate([held[r], v], axis=0).astype(bf16)
                    if r == 1 and keep is not None:
                        ls[keep, pl.ds(16 * (g // 2), 16), :] = v
                    lu[par, r, pl.ds(8 * (g // 2), 8), :] = pltpu.bitcast(v, u32)

            def conv(rows2, g, par, do_norm, keep, st):
                new = prep(rows2, g)
                parts = [S[g, j] for j in range(3)] + new
                for j in range(3):
                    S[g, j] = new[j]
                y = jnp.dot(up(L[g]), up(jnp.concatenate(parts, axis=0)), preferred_element_type=f32)
                if do_norm:
                    norm(1 - par, g, keep)
                Y[0, pl.ds(8 * g, 8), :] = y[0:8]
                Y[1, pl.ds(8 * g, 8), :] = y[8:16]
                y = tiles(y)
                s1, s2 = (y, y * y) if g % GS == 0 else (st[0] + y, st[1] + y * y)
                if g == GS - 1:
                    sa[0] = s1; sa[1] = s2
                elif g % GS == GS - 1:
                    sa[0] += s1; sa[1] += s2
                if g == G - 1:
                    red = []
                    for i in range(2):
                        p = [sa[i, pl.ds(j, 2 * NT, stride=8), :] for j in range(8)]
                        red.append((((p[0] + p[1]) + (p[2] + p[3])) + ((p[4] + p[5]) + (p[6] + p[7]))) * (1.0 / C))
                    v = jnp.maximum(red[1] - red[0] * red[0], 0.0)
                    rs = jax.lax.rsqrt(v * (1.0 / _ALPHA ** 2) + 1e-5 / _ALPHA ** 2)
                    for r in range(2):
                        mr[par, r] = jnp.concatenate([jnp.broadcast_to(rs[r * NT + t:r * NT + t + 1], (8, 128)) for t in range(NT)], axis=1)
                return s1, s2

            def mlp1(l, m0, M, b, pos, s):
                g = gelu(jnp.dot(up(w1t[pl.ds(m0 // 2, M // 2), :]), l, preferred_element_type=f32))
                if pos is not None:
                    gb = g.astype(bf16)
                    for c0 in range(0, M, 32):
                        q, o = divmod(m0 + c0, C)
                        hs[b, pos * (E // C) + q, pl.ds(o, 32), :] = gb[c0:c0 + 32]
                g2 = g * g
                for t in range(NT):
                    p = g2[:, t * 128:(t + 1) * 128]
                    s = p if s is None else s + p
                return s

            in0.wait()
            small[1].wait()
            w1f = w1_ref[...].astype(f32)
            w1t[...] = pk((w1f - jnp.mean(w1f, axis=0, keepdims=True)).T)
            for g in range(G):
                new = prep(xb.at[1, pl.ds(T - 6, 2)], g)
                for j in range(3):
                    S[g, j] = new[j]
            for k in range(2):
                sts = None
                for g in range(G):
                    sts = conv(xb.at[1, pl.ds(T - 4 + 2 * k, 2)], g, k, k == 1, None, sts)

            def block(b, _):
                @pl.when(b + 1 < NB - 1)
                def _():
                    in1(b + 1).start()
                @pl.when(b + 1 == NB - 1)
                def _():
                    in1_last.start()
                    xb[ls_, pl.ds(T - OFF, OFF)] = jnp.zeros((OFF, C, W), bf16)
                @pl.when(b < NB - 1)
                def _():
                    in1(b).wait()
                @pl.when(b == NB - 1)
                def _():
                    in2(0).start()
                    in1_last.wait()
                @pl.when(b == -(-NSP // NL))
                def _():
                    spill.start()
                @pl.when(b == QR // NL)
                def _():
                    spill.wait()
                M = E // 3
                for u in range(U):
                    keep = lslot(b, u + 1) if NA <= u + 1 < U else None
                    g = 0
                    sts = None
                    for st in range(3):
                        ss = None
                        for r in range(2):
                            ss = mlp1(up(lu[u % 2, r]), st * M, M, b, hpos(u, r), ss)
                            if r == 1:
                                acc[pl.ds(st * M, M), :] += ss
                            for _ in range(2):
                                sts = conv(xb.at[b % 2, pl.ds(2 * u, 2)], g, u % 2, True, keep, sts)
                                g += 1
                return 0
            jax.lax.fori_loop(0, NB, block, 0)

        pl.run_scoped(
            phase1,
            pltpu.VMEM((2, 2, C // 2, W), u32),
            pltpu.VMEM((2, 16 * NT, 128), f32),
            pltpu.VMEM((2, 2, 8, W), f32),
            pltpu.VMEM((G, 3, 8, W), u32),
            pltpu.VMEM((2, C, W), f32),
            pltpu.VMEM((G, 8, 96), u32),
        )

        def phase2(w2s, bias):
            for cp in small[2:]:
                cp.wait()
            sc = 1.0 / (2.0 * _ALPHA)
            ss = jnp.sum(acc[...].T, axis=0, keepdims=True) * (sc * sc)
            gx = jnp.sqrt(ss + 1e-6)
            nx = gx / (jnp.mean(gx, axis=-1, keepdims=True) + 1e-6)
            s = (g_ref[...].astype(f32).reshape(1, E) * nx + 1.0) * sc
            w2f = w2t_ref[...].astype(f32)
            w2s[...] = pk(w2f * s)
            bias[...] = jnp.broadcast_to(jnp.sum(w2f * b_ref[...].astype(f32).reshape(1, E), axis=1, keepdims=True), (C, 128))

            def block(parked, n, _):
                b = NB - 1 - n
                slot = (NB + n) % 2
                @pl.when(n <= K)
                def _():
                    in2(n + 1).start()
                @pl.when(jnp.logical_and(n >= 1, n + K + 1 < NB))
                def _():
                    far(n + K + 1).start()
                sent = lambda m: jnp.clip(2 * (m - N0 + 1), 0, jnp.maximum(m, 0))
                for i in range(2):
                    @pl.when(sent(n - 1) + i < sent(n))
                    def _():
                        out2(sent(n - 1) + i).start()
                @pl.when(jnp.logical_and(n >= 3, n < NRF + 3))
                def _():
                    back(n - 3).wait()
                @pl.when(jnp.logical_and(n >= 1, n < NRF + 1))
                def _():
                    back(n - 1).start(priority=PB)
                (far if parked else in2)(n).wait()
                def fin(h, r):
                    o = jnp.dot(up(w2s[...]), h, preferred_element_type=f32)
                    o = o + jnp.tile(bias[...], (1, NT)) + (hs[b + K + 2, T + r] if parked else xb[slot, r]).astype(f32)
                    hs[b, r] = o.astype(bf16)
                kept = lambda pos: hs[b, pl.ds(pos * (E // C), E // C)].reshape(E, W)
                for u in range(U):
                    if u < NA:
                        fin(kept(hpos(u, 0)), 2 * u)
                        fin(kept(hpos(u, 1)), 2 * u + 1)
                    else:
                        g = gelu(jnp.dot(up(w1t[...]), ls[lslot(b, u)], preferred_element_type=f32)).astype(bf16)
                        fin(kept(hpos(u, 0)), 2 * u)
                        fin(g, 2 * u + 1)
                return 0
            jax.lax.fori_loop(0, K + 2, functools.partial(block, False), 0)
            jax.lax.fori_loop(K + 2, NB, functools.partial(block, True), 0)
            out2(NB - 1).start()
            for n in range(NB):
                out2(n).wait()

        pl.run_scoped(phase2, pltpu.VMEM((C // 2, E), u32), pltpu.VMEM((C, 128), f32))

    scratch = [
        pltpu.VMEM((NB, (U + NA) * (E // C), C, W), bf16),
        pltpu.VMEM((QR, C, W), bf16),
        pltpu.VMEM((2, T, C, W), bf16),
        pltpu.VMEM((E // 2, C), u32),
        pltpu.VMEM((E, 128), f32),
        pltpu.SemaphoreType.DMA((2,)),
        pltpu.SemaphoreType.DMA((2,)),
        pltpu.SemaphoreType.DMA((NB,)),
        pltpu.VMEM((C, E), bf16),
        pltpu.VMEM((C, E), bf16),
        pltpu.VMEM((4, 3, C), bf16),
        pltpu.VMEM((E,), bf16),
        pltpu.VMEM((E,), bf16),
        pltpu.SemaphoreType.DMA((5,)),
    ]
    return kern, scratch

@jax.jit
def pallas_standalone__modern_conv_block_convnext_v2__vision_kernel(x, dw, w1, w2, grn_gamma, grn_beta):
    B, H, W, C = x.shape
    E = w1.shape[1]
    xt = jnp.transpose(x[0], (0, 2, 1))
    vm = pl.BlockSpec(memory_space=pltpu.VMEM)
    kern, scratch = make(H, W, C, E)
    out = pl.pallas_call(
        kern,
        in_specs=[pl.BlockSpec(memory_space=pl.ANY)] * 6,
        out_specs=pl.BlockSpec(memory_space=pl.ANY),
        out_shape=jax.ShapeDtypeStruct((H, C, W), x.dtype),
        scratch_shapes=scratch,
        compiler_params=pltpu.CompilerParams(vmem_limit_bytes=VL * 1024 * 1024, internal_scratch_in_bytes=ISB * 1024 if ISB else None),
    )(xt, dw, w1, w2.T, grn_gamma, grn_beta)
    return jnp.transpose(out, (0, 2, 1))[None]
```

```python
import jax
import jax.numpy as jnp
import numpy as np
import jax.experimental.pallas as pl
import jax.experimental.pallas.tpu as pltpu

_C0 = float(np.sqrt(2.0 / np.pi))
_ALPHA = float((_C0 * 0.044715) ** (1.0 / 3.0))
_A = _C0 / _ALPHA

_PAIRS = 8
_BACK_ROWS = 4
_BACK_STEPS = 18
_TAIL_CUTS = (0, 4, 7, _PAIRS)


def _gelu(u):
    return (jnp.tanh(u * (u * u + _A)) + 1.0) * u


def _make_kernel(H, W, C, E, back_steps=_BACK_STEPS):
    f32, bf16, u32, i32 = jnp.float32, jnp.bfloat16, jnp.uint32, jnp.int32
    U = _PAIRS
    T = 2 * U
    NB = H // T
    G = C // 8
    NT = W // 128
    HS = E // C
    NL = U - 1
    PARK = _BACK_ROWS * back_steps
    LCAP = NB * NL - PARK
    NR = NB // 2 + 1
    LEAD = 5
    M = E // 3
    park_start = pl.cdiv(PARK, NL)
    park_wait = LCAP // NL
    back_wait = NB - 1 - (PARK - 1) // NL
    assert H % (2 * T) == 0 and W == 512 and C == 96 and E == 4 * C
    assert _BACK_ROWS <= NL and park_start < park_wait < NB
    assert back_steps <= back_wait and NR <= back_wait < NB - 1

    def pack(v):
        return pltpu.bitcast(v.astype(bf16), u32)

    def unpack(v):
        return pltpu.bitcast(v, bf16)

    def h_pos(u, r):
        if u == 0:
            return r
        return u + 1 if r == 0 else None

    def ln_slot(b, u):
        i = b * NL + (u - 1)
        return jnp.where(i >= LCAP, i - LCAP, i)

    def kernel(x_hbm, dw_hbm, w1_hbm, w2t_hbm, gamma_hbm, beta_hbm, o_hbm,
               hs, ls, xb, w1t, ssq, w1_ref, w2t_ref, dw_ref, gamma_ref, beta_ref,
               xsem, lsem, osem, wsem):
        copy = pltpu.make_async_copy
        params = [copy(src, dst, wsem.at[i]) for i, (src, dst) in enumerate([
            (dw_hbm, dw_ref.at[pl.ds(0, 3)]), (w1_hbm, w1_ref), (w2t_hbm, w2t_ref),
            (gamma_hbm, gamma_ref), (beta_hbm, beta_ref)])]

        x_first = copy(x_hbm.at[pl.ds(0, LEAD)], xb.at[1, pl.ds(T - LEAD, LEAD)], xsem.at[1])
        x_final = copy(x_hbm.at[pl.ds(H - T + LEAD, T - LEAD)],
                       xb.at[1, pl.ds(0, T - LEAD)], xsem.at[1])

        def x_conv(b):
            return copy(x_hbm.at[pl.ds(b * T + LEAD, T)], xb.at[b % 2], xsem.at[b % 2])

        def x_near(n):
            return copy(x_hbm.at[pl.ds((NB - 1 - n) * T, T)], xb.at[n % 2], xsem.at[n % 2])

        def x_far(n):
            return copy(x_hbm.at[pl.ds((NB - 1 - n) * T, T)],
                        hs.at[NB - 1 - n + NR, pl.ds(T, T)], osem.at[n])

        def write(n):
            b = NB - 1 - n
            return copy(hs.at[b, pl.ds(0, T)], o_hbm.at[pl.ds(b * T, T)], osem.at[n])

        parked = ls.at[pl.ds(0, PARK)]
        park = copy(parked, o_hbm.at[pl.ds(0, PARK)], lsem.at[0])

        def read_back(n):
            @pl.when(jnp.logical_and(n >= 1, n <= back_steps))
            def _():
                rows = pl.ds(PARK - _BACK_ROWS * n, _BACK_ROWS)
                copy(o_hbm.at[rows], ls.at[rows], lsem.at[0]).start(priority=1)

        def pass1(ln, sums, stats, prev, ybuf, band):
            params[0].start()
            x_first.start()
            for cp in params[1:]:
                cp.start()
            x_conv(0).start()
            xb[1, T - LEAD - 1] = jnp.zeros((C, W), bf16)
            ssq[...] = jnp.zeros_like(ssq)

            params[0].wait()
            tap = jax.lax.broadcasted_iota(i32, (16, C), 0)
            taps = jnp.zeros((16, C), f32)
            for i in range(3):
                dwi = dw_ref[i].astype(f32)
                for j in range(3):
                    taps = jnp.where(tap == 3 * i + j, dwi[j:j + 1], taps)
            taps = taps.T.astype(bf16)
            tap = jax.lax.broadcasted_iota(i32, (16, 96), 0)
            col = jax.lax.broadcasted_iota(i32, (16, 96), 1)
            pair = (col >= 48).astype(i32)
            in_row = 2 * pair + ((col >> 3) & 1)
            shift = (col - 48 * pair) >> 4
            same = ((jax.lax.broadcasted_iota(i32, (C, 96), 0) & 7)
                    == (jax.lax.broadcasted_iota(i32, (C, 96), 1) & 7))
            rows = []
            for o in range(2):
                pick = jnp.logical_and(tap == (in_row - o) * 3 + shift, tap < 9)
                spread = jnp.dot(taps, pick.astype(f32).astype(bf16), preferred_element_type=f32)
                rows.append(jnp.where(same, spread, 0.0))
            for g in range(G):
                band[g] = pack(jnp.concatenate([v[8 * g:8 * g + 8] for v in rows], axis=0))

            lane = jax.lax.broadcasted_iota(i32, (8, 128), 1)
            first, last = lane == 0, lane == 127

            def shifted(x2, g):
                mid = pltpu.bitcast(x2[:, pl.ds(8 * g, 8), :].reshape(16, W), u32)
                tiles = [mid[:, 128 * t:128 * (t + 1)] for t in range(NT)]
                zero = jnp.zeros((8, 128), u32)
                up = [zero] + [pltpu.roll(v, 1, 1) for v in tiles]
                down = [pltpu.roll(v, 127, 1) for v in tiles] + [zero]
                left = [jnp.where(first, up[t], up[t + 1]) for t in range(NT)]
                right = [jnp.where(last, down[t + 1], down[t]) for t in range(NT)]
                return [jnp.concatenate(left, axis=1), mid, jnp.concatenate(right, axis=1)]

            def norm(par, g, keep):
                for r in range(2):
                    y = ybuf[r, pl.ds(8 * g, 16), :]
                    rstd, mean = stats[par, r], stats[2 + par, r]
                    v = jnp.concatenate(
                        [(y[0:8] - mean) * rstd, (y[8:16] - mean) * rstd], axis=0).astype(bf16)
                    if r == 1 and keep is not None:
                        ls[keep, pl.ds(8 * g, 16), :] = v
                    ln[par, r, pl.ds(4 * g, 8), :] = pltpu.bitcast(v, u32)

            def conv(x2, g0, par, norm_prev, keep):
                for g in (g0, g0 + 1):
                    new = shifted(x2, g)
                    window = [prev[g, j] for j in range(3)] + new
                    for j in range(3):
                        prev[g, j] = new[j]
                    y = jnp.dot(unpack(band[g]), unpack(jnp.concatenate(window, axis=0)),
                                preferred_element_type=f32)
                    if norm_prev and g == g0:
                        norm(1 - par, g0, keep)
                    for r in range(2):
                        ybuf[r, pl.ds(8 * g, 8), :] = y[8 * r:8 * r + 8]
                    y = jnp.concatenate([y[8 * r:8 * r + 8, 128 * t:128 * (t + 1)]
                                         for r in range(2) for t in range(NT)], axis=0)
                    s1, s2 = (y, y * y) if g == g0 else (s1 + y, s2 + y * y)
                if g0 == 0:
                    sums[0], sums[1] = s1, s2
                else:
                    sums[0] += s1
                    sums[1] += s2
                if g0 + 2 == G:
                    moments = []
                    for i in range(2):
                        p = [sums[i, pl.ds(j, 2 * NT, stride=8), :] for j in range(8)]
                        total = ((p[0] + p[1]) + (p[2] + p[3])) + ((p[4] + p[5]) + (p[6] + p[7]))
                        moments.append(total * (1.0 / C))
                    mean = moments[0]
                    var = jnp.maximum(moments[1] - mean * mean, 0.0)
                    rstd = jax.lax.rsqrt(var * (1.0 / _ALPHA ** 2) + 1e-5 / _ALPHA ** 2)
                    for r in range(2):
                        for slot, v in ((par, rstd), (2 + par, mean)):
                            stats[slot, r] = jnp.concatenate(
                                [jnp.broadcast_to(v[r * NT + t:r * NT + t + 1], (8, 128))
                                 for t in range(NT)], axis=1)

            def mlp(l, m0, b, pos, s):
                h = _gelu(jnp.dot(unpack(w1t[pl.ds(m0 // 2, M // 2), :]), l,
                                  preferred_element_type=f32))
                if pos is not None:
                    hb = h.astype(bf16)
                    for c in range(0, M, 32):
                        slab, o = divmod(m0 + c, C)
                        hs[b, pos * HS + slab, pl.ds(o, 32), :] = hb[c:c + 32]
                h2 = h * h
                for t in range(NT):
                    p = h2[:, 128 * t:128 * (t + 1)]
                    s = p if s is None else s + p
                return s

            x_first.wait()
            params[1].wait()
            w1t[...] = pack(w1_ref[...].astype(f32).T)
            for g in range(G):
                new = shifted(xb.at[1, pl.ds(T - 6, 2)], g)
                for j in range(3):
                    prev[g, j] = new[j]
            for k in range(2):
                for g in range(0, G, 2):
                    conv(xb.at[1, pl.ds(T - 4 + 2 * k, 2)], g, k, k == 1, None)

            def block(b, carry):
                pl.when(b + 1 < NB - 1)(lambda: x_conv(b + 1).start())

                @pl.when(b + 1 == NB - 1)
                def _():
                    x_final.start()
                    xb[1, pl.ds(T - LEAD, LEAD)] = jnp.zeros((LEAD, C, W), bf16)

                pl.when(b < NB - 1)(lambda: x_conv(b).wait())

                @pl.when(b == NB - 1)
                def _():
                    x_near(0).start()
                    x_final.wait()

                pl.when(b == park_start)(park.start)
                pl.when(b == park_wait)(park.wait)
                for u in range(U):
                    keep = ln_slot(b, u + 1) if u + 1 < U else None
                    for q in range(E // M):
                        s = None
                        for r in range(2):
                            s = mlp(unpack(ln[u % 2, r]), q * M, b, h_pos(u, r), s)
                            if r == 1:
                                ssq[pl.ds(q * M, M), :] += s
                            conv(xb.at[b % 2, pl.ds(2 * u, 2)], 4 * q + 2 * r, u % 2, True, keep)
                return carry

            jax.lax.fori_loop(0, NB, block, 0)

        pl.run_scoped(
            pass1,
            pltpu.VMEM((2, 2, C // 2, W), u32),
            pltpu.VMEM((2, 16 * NT, 128), f32),
            pltpu.VMEM((4, 2, 8, W), f32),
            pltpu.VMEM((G, 3, 8, W), u32),
            pltpu.VMEM((2, C, W), f32),
            pltpu.VMEM((G, 8, 96), u32),
        )

        def pass2(w2s, bias):
            for cp in params[2:]:
                cp.wait()
            unscale = 1.0 / (2.0 * _ALPHA)
            gx = jnp.sqrt(jnp.sum(ssq[...].T, axis=0, keepdims=True) * unscale ** 2 + 1e-6)
            nx = gx / (jnp.mean(gx, axis=-1, keepdims=True) + 1e-6)
            w2t = w2t_ref[...].astype(f32)
            scale = (gamma_ref[...].astype(f32).reshape(1, E) * nx + 1.0) * unscale
            w2s[...] = pack(w2t * scale)
            shift = jnp.sum(w2t * beta_ref[...].astype(f32).reshape(1, E), axis=1, keepdims=True)
            bias[...] = jnp.broadcast_to(shift, (C, 128))

            def compute(b, x_row, u0, u1):
                def finish(h, row):
                    o = jnp.dot(unpack(w2s[...]), h, preferred_element_type=f32)
                    o = o + jnp.tile(bias[...], (1, NT)) + x_row(row).astype(f32)
                    hs[b, row] = o.astype(bf16)

                def kept(u, r):
                    return hs[b, pl.ds(h_pos(u, r) * HS, HS)].reshape(E, W)

                for u in range(u0, u1):
                    if u == 0:
                        finish(kept(u, 0), 0)
                        finish(kept(u, 1), 1)
                    else:
                        h = _gelu(jnp.dot(unpack(w1t[...]), ls[ln_slot(b, u)],
                                          preferred_element_type=f32)).astype(bf16)
                        finish(kept(u, 0), 2 * u)
                        finish(h, 2 * u + 1)

            def read_step(n, carry):
                pl.when(n + 1 < NR)(lambda: x_near(n + 1).start())
                pl.when(jnp.logical_and(n >= 1, n + 1 < NR))(lambda: x_far(n - 1 + NR).start())
                read_back(n)

                @pl.when(n + 1 == NR)
                def _():
                    write(0).start()
                    write(1).start()

                x_near(n).wait()
                compute(NB - 1 - n, lambda row: xb[n % 2, row], 0, U)
                return carry

            def write_step(n, carry):
                write(2 * (n - NR + 1)).start()
                write(2 * (n - NR + 1) + 1).start()
                read_back(n)
                pl.when(n == back_wait)(lambda: copy(parked, parked, lsem.at[0]).wait())
                x_far(n).wait()
                compute(NB - 1 - n, lambda row: hs[NB - 1 - n + NR, T + row], 0, U)
                return carry

            jax.lax.fori_loop(0, NR, read_step, 0)
            jax.lax.fori_loop(NR, NB - 1, write_step, 0)
            write(NB - 2).start()
            x_far(NB - 1).wait()
            tail = []
            for u0, u1 in zip(_TAIL_CUTS[:-1], _TAIL_CUTS[1:]):
                compute(0, lambda row: hs[NR, T + row], u0, u1)
                rows = pl.ds(2 * u0, 2 * (u1 - u0))
                tail.append(copy(hs.at[0, rows], o_hbm.at[rows], osem.at[NB - 1]))
                tail[-1].start()
            for n in range(NB - 1):
                write(n).wait()
            for cp in tail:
                cp.wait()

        pl.run_scoped(pass2, pltpu.VMEM((C // 2, E), u32), pltpu.VMEM((C, 128), f32))

    scratch = [
        pltpu.VMEM((NB, (U + 1) * HS, C, W), bf16),
        pltpu.VMEM((LCAP, C, W), bf16),
        pltpu.VMEM((2, T, C, W), bf16),
        pltpu.VMEM((E // 2, C), u32),
        pltpu.VMEM((E, 128), f32),
        pltpu.VMEM((C, E), bf16),
        pltpu.VMEM((C, E), bf16),
        pltpu.VMEM((4, 3, C), bf16),
        pltpu.VMEM((E,), bf16),
        pltpu.VMEM((E,), bf16),
        pltpu.SemaphoreType.DMA((2,)),
        pltpu.SemaphoreType.DMA((1,)),
        pltpu.SemaphoreType.DMA((NB,)),
        pltpu.SemaphoreType.DMA((5,)),
    ]
    return kernel, scratch


@jax.jit
def pallas_standalone__modern_conv_block_convnext_v2__vision_kernel(
    x: jax.Array,
    dw: jax.Array,
    w1: jax.Array,
    w2: jax.Array,
    grn_gamma: jax.Array,
    grn_beta: jax.Array,
):
    B, H, W, C = x.shape
    assert B == 1 and dw.shape == (3, 3, C)
    kernel, scratch = _make_kernel(H, W, C, w1.shape[1])
    out = pl.pallas_call(
        kernel,
        in_specs=[pl.BlockSpec(memory_space=pl.ANY)] * 6,
        out_specs=pl.BlockSpec(memory_space=pl.ANY),
        out_shape=jax.ShapeDtypeStruct((H, C, W), x.dtype),
        scratch_shapes=scratch,
        compiler_params=pltpu.CompilerParams(vmem_limit_bytes=128 * 1024 * 1024),
    )(jnp.transpose(x[0], (0, 2, 1)), dw, w1, w2.T, grn_gamma, grn_beta)
    return jnp.transpose(out, (0, 2, 1))[None]
```

```python
import jax
import jax.numpy as jnp
import numpy as np
import jax.experimental.pallas as pl
import jax.experimental.pallas.tpu as pltpu

_C0 = float(np.sqrt(2.0 / np.pi))
_ALPHA = float((_C0 * 0.044715) ** (1.0 / 3.0))
_A = _C0 / _ALPHA

_PAIRS = 8
_RESIDENT = 19
_TAIL_CUTS = (0, 4, 7, _PAIRS)


def _gelu(u):
    return (jnp.tanh(u * (u * u + _A)) + 1.0) * u


def _make_kernel(H, W, C, E, resident=_RESIDENT):
    f32, bf16, u32, i32 = jnp.float32, jnp.bfloat16, jnp.uint32, jnp.int32
    U = _PAIRS
    T = 2 * U
    NB = H // T
    G = C // 8
    NT = W // 128
    HS = E // C
    NP = NB - resident
    NR = NB // 2 + 1
    LEAD = 5
    M = E // 3
    assert H % (2 * T) == 0 and W == 512 and C == 96 and E == 4 * C
    assert 0 < NP < NR <= resident

    def pack(v):
        return pltpu.bitcast(v.astype(bf16), u32)

    def unpack(v):
        return pltpu.bitcast(v, bf16)

    def h_pos(u, r):
        if r == 0:
            return u
        return U if u == 0 else None

    def ln_slot(b):
        return jnp.where(b >= resident, b - resident, b)

    def kernel(x_hbm, dw_hbm, w1_hbm, w2t_hbm, gamma_hbm, beta_hbm, o_hbm,
               hs, ls, xb, w1t, ssq, w1_ref, w2t_ref, dw_ref, gamma_ref, beta_ref,
               xsem, lsem, osem, wsem):
        copy = pltpu.make_async_copy
        params = [copy(src, dst, wsem.at[i]) for i, (src, dst) in enumerate([
            (dw_hbm, dw_ref.at[pl.ds(0, 3)]), (w1_hbm, w1_ref), (w2t_hbm, w2t_ref),
            (gamma_hbm, gamma_ref), (beta_hbm, beta_ref)])]

        x_first = copy(x_hbm.at[pl.ds(0, LEAD)], xb.at[1, pl.ds(T - LEAD, LEAD)], xsem.at[1])
        x_final = copy(x_hbm.at[pl.ds(H - T + LEAD, T - LEAD)],
                       xb.at[1, pl.ds(0, T - LEAD)], xsem.at[1])

        def x_conv(b):
            return copy(x_hbm.at[pl.ds(b * T + LEAD, T)], xb.at[b & 1], xsem.at[b & 1])

        def x_near(n):
            return copy(x_hbm.at[pl.ds((NB - 1 - n) * T, T)], xb.at[n & 1], xsem.at[n & 1])

        def x_far(n):
            return copy(x_hbm.at[pl.ds((NB - 1 - n) * T, T)],
                        hs.at[NB - 1 - n + NR, pl.ds(T, T)], osem.at[n])

        def write(n, k):
            blocks = pl.ds(NB - k - n, k)
            return copy(hs.at[blocks, pl.ds(0, T)], o_hbm.at[blocks], osem.at[n])

        def park(b):
            return copy(ls.at[b], o_hbm.at[b, pl.ds(0, U)], lsem.at[b])

        def unpark(b):
            return copy(o_hbm.at[b, pl.ds(0, U)], ls.at[b], lsem.at[b])

        def pass1(ln, sums, stats, prev, ybuf, band):
            params[0].start()
            x_first.start()
            params[1].start()
            x_conv(0).start()
            xb[1, T - LEAD - 1] = jnp.zeros((C, W), bf16)
            ssq[...] = jnp.zeros_like(ssq)

            params[0].wait()
            tap = jax.lax.broadcasted_iota(i32, (16, C), 0)
            taps = jnp.zeros((16, C), f32)
            for i in range(3):
                dwi = dw_ref[i].astype(f32)
                for j in range(3):
                    taps = jnp.where(tap == 3 * i + j, dwi[j:j + 1], taps)
            taps = taps.T.astype(bf16)
            tap = jax.lax.broadcasted_iota(i32, (16, 96), 0)
            col = jax.lax.broadcasted_iota(i32, (16, 96), 1)
            pair = (col >= 48).astype(i32)
            in_row = 2 * pair + ((col >> 3) & 1)
            shift = (col - 48 * pair) >> 4
            same = ((jax.lax.broadcasted_iota(i32, (C, 96), 0) & 7)
                    == (jax.lax.broadcasted_iota(i32, (C, 96), 1) & 7))
            rows = []
            for o in range(2):
                pick = jnp.logical_and(tap == (in_row - o) * 3 + shift, tap < 9)
                spread = jnp.dot(taps, pick.astype(f32).astype(bf16), preferred_element_type=f32)
                rows.append(jnp.where(same, spread, 0.0))
            for g in range(G):
                band[g] = pack(jnp.concatenate([v[8 * g:8 * g + 8] for v in rows], axis=0))

            lane = jax.lax.broadcasted_iota(i32, (8, 128), 1)
            first, last = lane == 0, lane == 127

            def shifted(x2, g):
                mid = pltpu.bitcast(x2[:, pl.ds(8 * g, 8), :].reshape(16, W), u32)
                tiles = [mid[:, 128 * t:128 * (t + 1)] for t in range(NT)]
                zero = jnp.zeros((8, 128), u32)
                up = [zero] + [pltpu.roll(v, 1, 1) for v in tiles]
                down = [pltpu.roll(v, 127, 1) for v in tiles] + [zero]
                left = [jnp.where(first, up[t], up[t + 1]) for t in range(NT)]
                right = [jnp.where(last, down[t + 1], down[t]) for t in range(NT)]
                return [jnp.concatenate(left, axis=1), mid, jnp.concatenate(right, axis=1)]

            def norm(par, g, keep):
                for r in range(2):
                    y = ybuf[r, pl.ds(8 * g, 16), :]
                    rstd, mean = stats[par, r], stats[2 + par, r]
                    v = jnp.concatenate(
                        [(y[0:8] - mean) * rstd, (y[8:16] - mean) * rstd], axis=0).astype(bf16)
                    if r == 1 and keep is not None:
                        keep[pl.ds(8 * g, 16), :] = v
                    ln[par, r, pl.ds(4 * g, 8), :] = pltpu.bitcast(v, u32)

            def conv(x2, g0, par, norm_prev, keep):
                for g in (g0, g0 + 1):
                    new = shifted(x2, g)
                    window = [prev[g, j] for j in range(3)] + new
                    for j in range(3):
                        prev[g, j] = new[j]
                    y = jnp.dot(unpack(band[g]), unpack(jnp.concatenate(window, axis=0)),
                                preferred_element_type=f32)
                    if norm_prev and g == g0:
                        norm(1 - par, g0, keep)
                    for r in range(2):
                        ybuf[r, pl.ds(8 * g, 8), :] = y[8 * r:8 * r + 8]
                    y = jnp.concatenate([y[8 * r:8 * r + 8, 128 * t:128 * (t + 1)]
                                         for r in range(2) for t in range(NT)], axis=0)
                    s1, s2 = (y, y * y) if g == g0 else (s1 + y, s2 + y * y)
                if g0 == 0:
                    sums[0], sums[1] = s1, s2
                else:
                    sums[0] += s1
                    sums[1] += s2
                if g0 + 2 == G:
                    moments = []
                    for i in range(2):
                        p = [sums[i, pl.ds(j, 2 * NT, stride=8), :] for j in range(8)]
                        total = ((p[0] + p[1]) + (p[2] + p[3])) + ((p[4] + p[5]) + (p[6] + p[7]))
                        moments.append(total * (1.0 / C))
                    mean = moments[0]
                    var = jnp.maximum(moments[1] - mean * mean, 0.0)
                    rstd = jax.lax.rsqrt(var * (1.0 / _ALPHA ** 2) + 1e-5 / _ALPHA ** 2)
                    for r in range(2):
                        for slot, v in ((par, rstd), (2 + par, mean)):
                            stats[slot, r] = jnp.concatenate(
                                [jnp.broadcast_to(v[r * NT + t:r * NT + t + 1], (8, 128))
                                 for t in range(NT)], axis=1)

            def mlp(l, m0, dst, width, s):
                h = _gelu(jnp.dot(unpack(w1t[pl.ds(m0 // 2, M // 2), :]), l,
                                  preferred_element_type=f32))
                if m0 < width:
                    hb = h[:width - m0].astype(bf16)
                    for c in range(0, hb.shape[0], 32):
                        slab, o = divmod(m0 + c, C)
                        dst[slab, pl.ds(o, 32), :] = hb[c:c + 32]
                h2 = h * h
                for t in range(NT):
                    p = h2[:, 128 * t:128 * (t + 1)]
                    s = p if s is None else s + p
                return s

            x_first.wait()
            params[1].wait()
            w1t[...] = pack(w1_ref[...].astype(f32).T)
            for g in range(G):
                new = shifted(xb.at[1, pl.ds(T - 6, 2)], g)
                for j in range(3):
                    prev[g, j] = new[j]
            for k in range(2):
                for g in range(0, G, 2):
                    conv(xb.at[1, pl.ds(T - 4 + 2 * k, 2)], g, k, k == 1, None)

            def block(b, carry):
                pl.when(b + 1 < NB - 1)(lambda: x_conv(b + 1).start())

                @pl.when(b + 1 == NB - 1)
                def _():
                    x_final.start()
                    xb[1, pl.ds(T - LEAD, LEAD)] = jnp.zeros((LEAD, C, W), bf16)

                pl.when(b < NB - 1)(lambda: x_conv(b).wait())

                @pl.when(b == NB - 1)
                def _():
                    x_near(0).start()
                    for cp in params[2:]:
                        cp.start()
                    x_final.wait()

                pl.when(jnp.logical_and(b >= 1, b <= NP))(lambda: park(b - 1).start())
                pl.when(b >= resident)(lambda: park(b - resident).wait())
                lsb = ls.at[ln_slot(b)]
                for u in range(U):
                    keep = lsb.at[u] if u + 1 < U else None
                    for q in range(E // M):
                        s = None
                        for r in range(2):
                            if h_pos(u, r) is not None:
                                dst, width = hs.at[b, pl.ds(h_pos(u, r) * HS, HS)], E
                            else:
                                dst, width = lsb.at[pl.ds(U - 1, 1)], C * (u == U - 1)
                            s = mlp(unpack(ln[u % 2, r]), q * M, dst, width, s)
                            if r == 1:
                                ssq[pl.ds(q * M, M), :] += s
                            conv(xb.at[b & 1, pl.ds(2 * u, 2)], 4 * q + 2 * r, u % 2, True, keep)
                return carry

            jax.lax.fori_loop(0, NB, block, 0)

        pl.run_scoped(
            pass1,
            pltpu.VMEM((2, 2, C // 2, W), u32),
            pltpu.VMEM((2, 16 * NT, 128), f32),
            pltpu.VMEM((4, 2, 8, W), f32),
            pltpu.VMEM((G, 3, 8, W), u32),
            pltpu.VMEM((2, C, W), f32),
            pltpu.VMEM((G, 8, 96), u32),
        )

        def pass2(w2s, bias):
            for cp in params[2:]:
                cp.wait()
            unscale = 1.0 / (2.0 * _ALPHA)
            gx = jnp.sqrt(jnp.sum(ssq[...].T, axis=0, keepdims=True) * unscale ** 2 + 1e-6)
            nx = gx / (jnp.mean(gx, axis=-1, keepdims=True) + 1e-6)
            w2t = w2t_ref[...].astype(f32)
            scale = (gamma_ref[...].astype(f32).reshape(1, E) * nx + 1.0) * unscale
            w2s[...] = pack(w2t * scale)
            shift = jnp.sum(w2t * beta_ref[...].astype(f32).reshape(1, E), axis=1, keepdims=True)
            bias[...] = jnp.broadcast_to(shift, (C, 128))

            def compute(b, x_row, u0, u1):
                def finish(h, row):
                    o = jnp.dot(unpack(w2s[...]), h, preferred_element_type=f32)
                    o = o + jnp.tile(bias[...], (1, NT)) + x_row(row).astype(f32)
                    hs[b, row] = o.astype(bf16)

                def kept(u, r):
                    return hs[b, pl.ds(h_pos(u, r) * HS, HS)].reshape(E, W)

                lsb = ls.at[ln_slot(b)]
                for u in range(max(u0, 1), u1):
                    m0 = C * (u == U - 1)
                    h = _gelu(jnp.dot(unpack(w1t[pl.ds(m0 // 2, (E - m0) // 2), :]), lsb[u - 1],
                                      preferred_element_type=f32)).astype(bf16)
                    if m0:
                        h = jnp.concatenate([lsb[U - 1], h], axis=0)
                    if u == 1:
                        finish(kept(0, 0), 0)
                        finish(kept(0, 1), 1)
                    finish(kept(u, 0), 2 * u)
                    finish(h, 2 * u + 1)

            def read_step(n, carry):
                pl.when(n + 1 < NR)(lambda: x_near(n + 1).start())
                pl.when(jnp.logical_and(n >= 1, n + 1 < NR))(lambda: x_far(n - 1 + NR).start())
                pl.when(jnp.logical_and(n >= 1, n <= NP))(
                    lambda: unpark(NP - n).start(priority=1))
                pl.when(n + 1 == NR)(lambda: write(0, 2).start())
                x_near(n).wait()
                compute(NB - 1 - n, lambda row: xb[n & 1, row], 0, U)
                return carry

            def write_step(n, carry):
                write(2 * (n - NR + 1), 2).start()
                pl.when(n >= resident)(lambda: unpark(NB - 1 - n).wait())
                x_far(n).wait()
                compute(NB - 1 - n, lambda row: hs[NB - 1 - n + NR, T + row], 0, U)
                return carry

            jax.lax.fori_loop(0, NR, read_step, 0)
            jax.lax.fori_loop(NR, NB - 1, write_step, 0)
            write(NB - 2, 1).start()
            unpark(0).wait()
            x_far(NB - 1).wait()
            tail = []
            for u0, u1 in zip(_TAIL_CUTS[:-1], _TAIL_CUTS[1:]):
                compute(0, lambda row: hs[NR, T + row], u0, u1)
                rows = pl.ds(2 * u0, 2 * (u1 - u0))
                tail.append(copy(hs.at[0, rows], o_hbm.at[0, rows], osem.at[NB - 1]))
                tail[-1].start()
            for n in range(0, NB - 2, 2):
                write(n, 2).wait()
            write(NB - 2, 1).wait()
            for cp in tail:
                cp.wait()

        pl.run_scoped(pass2, pltpu.VMEM((C // 2, E), u32), pltpu.VMEM((C, 128), f32))

    scratch = [
        pltpu.VMEM((NB, (U + 1) * HS, C, W), bf16),
        pltpu.VMEM((resident, U, C, W), bf16),
        pltpu.VMEM((2, T, C, W), bf16),
        pltpu.VMEM((E // 2, C), u32),
        pltpu.VMEM((E, 128), f32),
        pltpu.VMEM((C, E), bf16),
        pltpu.VMEM((C, E), bf16),
        pltpu.VMEM((4, 3, C), bf16),
        pltpu.VMEM((E,), bf16),
        pltpu.VMEM((E,), bf16),
        pltpu.SemaphoreType.DMA((2,)),
        pltpu.SemaphoreType.DMA((NP,)),
        pltpu.SemaphoreType.DMA((NB,)),
        pltpu.SemaphoreType.DMA((5,)),
    ]
    return kernel, scratch


@jax.jit
def pallas_standalone__modern_conv_block_convnext_v2__vision_kernel(
    x: jax.Array,
    dw: jax.Array,
    w1: jax.Array,
    w2: jax.Array,
    grn_gamma: jax.Array,
    grn_beta: jax.Array,
):
    B, H, W, C = x.shape
    assert B == 1 and dw.shape == (3, 3, C)
    kernel, scratch = _make_kernel(H, W, C, w1.shape[1])
    out = pl.pallas_call(
        kernel,
        in_specs=[pl.BlockSpec(memory_space=pl.ANY)] * 6,
        out_specs=pl.BlockSpec(memory_space=pl.ANY),
        out_shape=jax.ShapeDtypeStruct((H // (2 * _PAIRS), 2 * _PAIRS, C, W), x.dtype),
        scratch_shapes=scratch,
        compiler_params=pltpu.CompilerParams(vmem_limit_bytes=128 * 1024 * 1024),
    )(jnp.transpose(x[0], (0, 2, 1)), dw, w1, w2.T, grn_gamma, grn_beta)
    return jnp.transpose(out.reshape(H, C, W), (0, 2, 1))[None]
```

```python
import jax
import jax.numpy as jnp
import numpy as np
import jax.experimental.pallas as pl
import jax.experimental.pallas.tpu as pltpu

_C0 = float(np.sqrt(2.0 / np.pi))
_ALPHA = float((_C0 * 0.044715) ** (1.0 / 3.0))
_A = _C0 / _ALPHA

_PAIRS = 8
_RESIDENT = 19
_TAIL_CUTS = (0, 3, 5, 7, _PAIRS)


def _gelu(u):
    return (jnp.tanh(u * (u * u + _A)) + 1.0) * u


def _make_kernel(H, W, C, E, resident=_RESIDENT):
    f32, bf16, u32, i32 = jnp.float32, jnp.bfloat16, jnp.uint32, jnp.int32
    U = _PAIRS
    T = 2 * U
    NB = H // T
    G = C // 8
    NT = W // 128
    HS = E // C
    NP = NB - resident
    NR = NB // 2 + 1
    LEAD = 5
    M = E // 3
    assert H % (2 * T) == 0 and W == 512 and C == 96 and E == 4 * C
    assert 0 < NP < NR <= resident

    def pack(v):
        return pltpu.bitcast(v.astype(bf16), u32)

    def unpack(v):
        return pltpu.bitcast(v, bf16)

    def h_pos(u, r):
        if r == 0:
            return u
        return U if u == 0 else None

    def ln_slot(b):
        return jnp.where(b >= resident, b - resident, b)

    def kernel(x_hbm, dw_hbm, w1_hbm, w2t_hbm, gamma_hbm, beta_hbm, o_hbm,
               hs, ls, xb, w1t, ssq, w1_ref, w2t_ref, dw_ref, gamma_ref, beta_ref,
               xsem, lsem, osem, wsem):
        copy = pltpu.make_async_copy
        params = [copy(src, dst, wsem.at[i]) for i, (src, dst) in enumerate([
            (dw_hbm, dw_ref.at[pl.ds(0, 3)]), (w1_hbm, w1_ref), (w2t_hbm, w2t_ref),
            (gamma_hbm, gamma_ref), (beta_hbm, beta_ref)])]

        x_first = copy(x_hbm.at[pl.ds(0, LEAD)], xb.at[1, pl.ds(T - LEAD, LEAD)], xsem.at[1])
        x_final = copy(x_hbm.at[pl.ds(H - T + LEAD, T - LEAD)],
                       xb.at[1, pl.ds(0, T - LEAD)], xsem.at[1])

        def x_conv(b):
            return copy(x_hbm.at[pl.ds(b * T + LEAD, T)], xb.at[b & 1], xsem.at[b & 1])

        def x_near(n):
            return copy(x_hbm.at[pl.ds((NB - 1 - n) * T, T)], xb.at[n & 1], xsem.at[n & 1])

        def x_far(n):
            return copy(x_hbm.at[pl.ds((NB - 1 - n) * T, T)],
                        hs.at[NB - 1 - n + NR, pl.ds(T, T)], osem.at[n])

        def write(n, k):
            blocks = pl.ds(NB - k - n, k)
            return copy(hs.at[blocks, pl.ds(0, T)], o_hbm.at[blocks], osem.at[n])

        def park(b):
            return copy(ls.at[b], o_hbm.at[b, pl.ds(0, U)], lsem.at[b])

        def unpark(b):
            return copy(o_hbm.at[b, pl.ds(0, U)], ls.at[b], lsem.at[b])

        def pass1(ln, sums, stats, prev, ybuf, band):
            params[0].start()
            x_first.start()
            for cp in params[1:]:
                cp.start()
            x_conv(0).start()
            xb[1, T - LEAD - 1] = jnp.zeros((C, W), bf16)
            ssq[...] = jnp.zeros_like(ssq)

            params[0].wait()
            tap = jax.lax.broadcasted_iota(i32, (16, C), 0)
            taps = jnp.zeros((16, C), f32)
            for i in range(3):
                dwi = dw_ref[i].astype(f32)
                for j in range(3):
                    taps = jnp.where(tap == 3 * i + j, dwi[j:j + 1], taps)
            taps = taps.T.astype(bf16)
            tap = jax.lax.broadcasted_iota(i32, (16, 96), 0)
            col = jax.lax.broadcasted_iota(i32, (16, 96), 1)
            pair = (col >= 48).astype(i32)
            in_row = 2 * pair + ((col >> 3) & 1)
            shift = (col - 48 * pair) >> 4
            same = ((jax.lax.broadcasted_iota(i32, (C, 96), 0) & 7)
                    == (jax.lax.broadcasted_iota(i32, (C, 96), 1) & 7))
            rows = []
            for o in range(2):
                pick = jnp.logical_and(tap == (in_row - o) * 3 + shift, tap < 9)
                spread = jnp.dot(taps, pick.astype(f32).astype(bf16), preferred_element_type=f32)
                rows.append(jnp.where(same, spread, 0.0))
            for g in range(G):
                band[g] = pack(jnp.concatenate([v[8 * g:8 * g + 8] for v in rows], axis=0))

            lane = jax.lax.broadcasted_iota(i32, (8, 128), 1)
            first, last = lane == 0, lane == 127

            def shifted(x2, g):
                mid = pltpu.bitcast(x2[:, pl.ds(8 * g, 8), :].reshape(16, W), u32)
                tiles = [mid[:, 128 * t:128 * (t + 1)] for t in range(NT)]
                zero = jnp.zeros((8, 128), u32)
                up = [zero] + [pltpu.roll(v, 1, 1) for v in tiles]
                down = [pltpu.roll(v, 127, 1) for v in tiles] + [zero]
                left = [jnp.where(first, up[t], up[t + 1]) for t in range(NT)]
                right = [jnp.where(last, down[t + 1], down[t]) for t in range(NT)]
                return [jnp.concatenate(left, axis=1), mid, jnp.concatenate(right, axis=1)]

            def norm(par, g, keep):
                for r in range(2):
                    y = ybuf[r, pl.ds(8 * g, 16), :]
                    rstd, mean = stats[par, r], stats[2 + par, r]
                    v = jnp.concatenate(
                        [(y[0:8] - mean) * rstd, (y[8:16] - mean) * rstd], axis=0).astype(bf16)
                    if r == 1 and keep is not None:
                        keep[pl.ds(8 * g, 16), :] = v
                    ln[par, r, pl.ds(4 * g, 8), :] = pltpu.bitcast(v, u32)

            def conv(x2, g0, par, norm_prev, keep):
                for g in (g0, g0 + 1):
                    new = shifted(x2, g)
                    window = [prev[g, j] for j in range(3)] + new
                    for j in range(3):
                        prev[g, j] = new[j]
                    y = jnp.dot(unpack(band[g]), unpack(jnp.concatenate(window, axis=0)),
                                preferred_element_type=f32)
                    if norm_prev and g == g0:
                        norm(1 - par, g0, keep)
                    for r in range(2):
                        ybuf[r, pl.ds(8 * g, 8), :] = y[8 * r:8 * r + 8]
                    y = jnp.concatenate([y[8 * r:8 * r + 8, 128 * t:128 * (t + 1)]
                                         for r in range(2) for t in range(NT)], axis=0)
                    s1, s2 = (y, y * y) if g == g0 else (s1 + y, s2 + y * y)
                if g0 == 0:
                    sums[0], sums[1] = s1, s2
                else:
                    sums[0] += s1
                    sums[1] += s2
                if g0 + 2 == G:
                    moments = []
                    for i in range(2):
                        p = [sums[i, pl.ds(j, 2 * NT, stride=8), :] for j in range(8)]
                        total = ((p[0] + p[1]) + (p[2] + p[3])) + ((p[4] + p[5]) + (p[6] + p[7]))
                        moments.append(total * (1.0 / C))
                    mean = moments[0]
                    var = jnp.maximum(moments[1] - mean * mean, 0.0)
                    rstd = jax.lax.rsqrt(var * (1.0 / _ALPHA ** 2) + 1e-5 / _ALPHA ** 2)
                    for r in range(2):
                        for slot, v in ((par, rstd), (2 + par, mean)):
                            stats[slot, r] = jnp.concatenate(
                                [jnp.broadcast_to(v[r * NT + t:r * NT + t + 1], (8, 128))
                                 for t in range(NT)], axis=1)

            def mlp(l, m0, dst, width, s):
                h = _gelu(jnp.dot(unpack(w1t[pl.ds(m0 // 2, M // 2), :]), l,
                                  preferred_element_type=f32))
                if m0 < width:
                    hb = h[:width - m0].astype(bf16)
                    for c in range(0, hb.shape[0], 32):
                        slab, o = divmod(m0 + c, C)
                        dst[slab, pl.ds(o, 32), :] = hb[c:c + 32]
                h2 = h * h
                for t in range(NT):
                    p = h2[:, 128 * t:128 * (t + 1)]
                    s = p if s is None else s + p
                return s

            x_first.wait()
            params[1].wait()
            w1t[...] = pack(w1_ref[...].astype(f32).T)
            for g in range(G):
                new = shifted(xb.at[1, pl.ds(T - 6, 2)], g)
                for j in range(3):
                    prev[g, j] = new[j]
            for k in range(2):
                for g in range(0, G, 2):
                    conv(xb.at[1, pl.ds(T - 4 + 2 * k, 2)], g, k, k == 1, None)

            def block(b, carry):
                pl.when(b + 1 < NB - 1)(lambda: x_conv(b + 1).start())

                @pl.when(b + 1 == NB - 1)
                def _():
                    x_final.start()
                    xb[1, pl.ds(T - LEAD, LEAD)] = jnp.zeros((LEAD, C, W), bf16)

                pl.when(b < NB - 1)(lambda: x_conv(b).wait())

                @pl.when(b == NB - 1)
                def _():
                    x_near(0).start()
                    x_final.wait()

                pl.when(jnp.logical_and(b >= 1, b <= NP))(lambda: park(b - 1).start())
                pl.when(b >= resident)(lambda: park(b - resident).wait())
                lsb = ls.at[ln_slot(b)]
                for u in range(U):
                    keep = lsb.at[u] if u + 1 < U else None
                    for q in range(E // M):
                        s = None
                        for r in range(2):
                            if h_pos(u, r) is not None:
                                dst, width = hs.at[b, pl.ds(h_pos(u, r) * HS, HS)], E
                            else:
                                dst, width = lsb.at[pl.ds(U - 1, 1)], C * (u == U - 1)
                            s = mlp(unpack(ln[u % 2, r]), q * M, dst, width, s)
                            if r == 1:
                                ssq[pl.ds(q * M, M), :] += s
                            conv(xb.at[b & 1, pl.ds(2 * u, 2)], 4 * q + 2 * r, u % 2, True, keep)
                return carry

            jax.lax.fori_loop(0, NB, block, 0)

        pl.run_scoped(
            pass1,
            pltpu.VMEM((2, 2, C // 2, W), u32),
            pltpu.VMEM((2, 16 * NT, 128), f32),
            pltpu.VMEM((4, 2, 8, W), f32),
            pltpu.VMEM((G, 3, 8, W), u32),
            pltpu.VMEM((2, C, W), f32),
            pltpu.VMEM((G, 8, 96), u32),
        )

        def pass2(w2s, bias):
            for cp in params[2:]:
                cp.wait()
            unscale = 1.0 / (2.0 * _ALPHA)
            gx = jnp.sqrt(jnp.sum(ssq[...].T, axis=0, keepdims=True) * unscale ** 2 + 1e-6)
            nx = gx / (jnp.mean(gx, axis=-1, keepdims=True) + 1e-6)
            w2t = w2t_ref[...].astype(f32)
            scale = (gamma_ref[...].astype(f32).reshape(1, E) * nx + 1.0) * unscale
            w2s[...] = pack(w2t * scale)
            shift = jnp.sum(w2t * beta_ref[...].astype(f32).reshape(1, E), axis=1, keepdims=True)
            bias[...] = jnp.broadcast_to(shift, (C, 128))

            def compute(b, x_row, u0, u1):
                def finish(h, row):
                    o = jnp.dot(unpack(w2s[...]), h, preferred_element_type=f32)
                    o = o + jnp.tile(bias[...], (1, NT)) + x_row(row).astype(f32)
                    hs[b, row] = o.astype(bf16)

                def kept(u, r):
                    return hs[b, pl.ds(h_pos(u, r) * HS, HS)].reshape(E, W)

                lsb = ls.at[ln_slot(b)]
                for u in range(max(u0, 1), u1):
                    m0 = C * (u == U - 1)
                    h = _gelu(jnp.dot(unpack(w1t[pl.ds(m0 // 2, (E - m0) // 2), :]), lsb[u - 1],
                                      preferred_element_type=f32)).astype(bf16)
                    if m0:
                        h = jnp.concatenate([lsb[U - 1], h], axis=0)
                    if u == 1:
                        finish(kept(0, 0), 0)
                        finish(kept(0, 1), 1)
                    finish(kept(u, 0), 2 * u)
                    finish(h, 2 * u + 1)

            def read_step(n, carry):
                pl.when(n + 1 < NR)(lambda: x_near(n + 1).start())
                pl.when(jnp.logical_and(n >= 1, n + 1 < NR))(lambda: x_far(n - 1 + NR).start())
                pl.when(jnp.logical_and(n >= 1, n <= NP))(
                    lambda: unpark(NP - n).start(priority=1))
                pl.when(n + 1 == NR)(lambda: write(0, 2).start())
                x_near(n).wait()
                compute(NB - 1 - n, lambda row: xb[n & 1, row], 0, U)
                return carry

            def write_step(n, carry):
                write(2 * (n - NR + 1), 2).start()
                pl.when(n >= resident)(lambda: unpark(NB - 1 - n).wait())
                x_far(n).wait()
                compute(NB - 1 - n, lambda row: hs[NB - 1 - n + NR, T + row], 0, U)
                return carry

            jax.lax.fori_loop(0, NR, read_step, 0)
            jax.lax.fori_loop(NR, NB - 1, write_step, 0)
            write(NB - 2, 1).start()
            unpark(0).wait()
            x_far(NB - 1).wait()
            tail = []
            for u0, u1 in zip(_TAIL_CUTS[:-1], _TAIL_CUTS[1:]):
                compute(0, lambda row: hs[NR, T + row], u0, u1)
                rows = pl.ds(2 * u0, 2 * (u1 - u0))
                tail.append(copy(hs.at[0, rows], o_hbm.at[0, rows], osem.at[NB - 1]))
                tail[-1].start()
            for n in range(0, NB - 2, 2):
                write(n, 2).wait()
            write(NB - 2, 1).wait()
            for cp in tail:
                cp.wait()

        pl.run_scoped(pass2, pltpu.VMEM((C // 2, E), u32), pltpu.VMEM((C, 128), f32))

    scratch = [
        pltpu.VMEM((NB, (U + 1) * HS, C, W), bf16),
        pltpu.VMEM((resident, U, C, W), bf16),
        pltpu.VMEM((2, T, C, W), bf16),
        pltpu.VMEM((E // 2, C), u32),
        pltpu.VMEM((E, 128), f32),
        pltpu.VMEM((C, E), bf16),
        pltpu.VMEM((C, E), bf16),
        pltpu.VMEM((4, 3, C), bf16),
        pltpu.VMEM((E,), bf16),
        pltpu.VMEM((E,), bf16),
        pltpu.SemaphoreType.DMA((2,)),
        pltpu.SemaphoreType.DMA((NP,)),
        pltpu.SemaphoreType.DMA((NB,)),
        pltpu.SemaphoreType.DMA((5,)),
    ]
    return kernel, scratch


@jax.jit
def pallas_standalone__modern_conv_block_convnext_v2__vision_kernel(
    x: jax.Array,
    dw: jax.Array,
    w1: jax.Array,
    w2: jax.Array,
    grn_gamma: jax.Array,
    grn_beta: jax.Array,
):
    B, H, W, C = x.shape
    assert B == 1 and dw.shape == (3, 3, C)
    kernel, scratch = _make_kernel(H, W, C, w1.shape[1])
    out = pl.pallas_call(
        kernel,
        in_specs=[pl.BlockSpec(memory_space=pl.ANY)] * 6,
        out_specs=pl.BlockSpec(memory_space=pl.ANY),
        out_shape=jax.ShapeDtypeStruct((H // (2 * _PAIRS), 2 * _PAIRS, C, W), x.dtype),
        scratch_shapes=scratch,
        compiler_params=pltpu.CompilerParams(vmem_limit_bytes=128 * 1024 * 1024),
    )(jnp.transpose(x[0], (0, 2, 1)), dw, w1, w2.T, grn_gamma, grn_beta)
    return jnp.transpose(out.reshape(H, C, W), (0, 2, 1))[None]
```
